```python
import os as _os
_os.environ.setdefault("JAX_PLATFORMS", "cpu")
import jax
import jax.numpy as jnp

def _softmax(x, axis=-1):
    return jax.nn.softmax(x, axis=axis)
def _gelu(x):
    return jax.nn.gelu(x, approximate=True)
def _silu(x):
    return jax.nn.silu(x)
def _sigmoid(x):
    return jax.nn.sigmoid(x)
def _layernorm(x, axis=-1, eps=1e-5):
    m = jnp.mean(x, axis=axis, keepdims=True)
    v = jnp.var(x, axis=axis, keepdims=True)
    return (x - m) / jnp.sqrt(v + eps)
def _scatter_add(tgt, idx, src, axis=0):
    return tgt.at[idx].add(src)
def _segment_sum(src, seg, n):
    return jax.ops.segment_sum(src, seg, n)
class _Rng:
    def __init__(self, key):
        self._k = key
    def _next(self):
        self._k, sub = jax.random.split(self._k)
        return sub
    def normal(self, shape):
        return jax.random.normal(self._next(), shape, dtype=jnp.bfloat16)
    def randint(self, lo, hi, shape):
        return jax.random.randint(self._next(), shape, lo, hi, dtype=jnp.int32)
    def uniform(self, shape, lo=0.0, hi=1.0):
        return jax.random.uniform(self._next(), shape, jnp.bfloat16, lo, hi)
    def permutation(self, n):
        return jax.random.permutation(self._next(), n)


kernel_name = 'interleave_layers__mha_block__dense_activation_gelu__prompt'

def setup_inputs():
    _rng = _Rng(jax.random.key(int.from_bytes(__import__("os").urandom(4), "little")))
    _w = (lambda a: (lambda t: t.astype(jnp.bfloat16) if jnp.issubdtype(t.dtype, jnp.floating) else t)(jnp.asarray(a)))
    def _A_setup():
        B, S, D, H = 1, 2048, 512, 32
        return {
            "x": _w((lambda *s: _rng.normal(s) * 0.05)(B, S, D)),
            "wqkv": _w((lambda *s: _rng.normal(s) * 0.05)(D, 3 * D)),
            "wo": _w((lambda *s: _rng.normal(s) * 0.05)(D, D)),
        }
    _A_in = _A_setup()

    def _B_setup():
        B, S, D, F = 1, 2048, 512, 1792
        return {
            "x": _w((lambda *s: _rng.normal(s) * 0.05)(B, S, D)),
            "w1": _w((lambda *s: _rng.normal(s) * 0.4)(D, F) * (D ** -0.5)),
            "b1": _w((lambda *s: _rng.normal(s) * 0.4)(F) * 0.01),
            "w2": _w((lambda *s: _rng.normal(s) * 0.4)(F, D) * (F ** -0.5)),
            "b2": _w((lambda *s: _rng.normal(s) * 0.4)(D) * 0.01),
        }
    _B_in = _B_setup()

    return {
        "A_x": _A_in["x"],
        "A_wqkv": _A_in["wqkv"],
        "A_wo": _A_in["wo"],
        "B_x": _B_in["x"],
        "B_w1": _B_in["w1"],
        "B_b1": _B_in["b1"],
        "B_w2": _B_in["w2"],
        "B_b2": _B_in["b2"],
    }

def reference(A_x, A_wqkv, A_wo, B_x, B_w1, B_b1, B_w2, B_b2):
    def _A_ref(x, wqkv, wo):
        B, S, D = x.shape
        H = 32
        Dh = D // H
        qkv = (lambda x, *d: x.transpose(*d))((x @ wqkv).reshape(B, S, 3, H, Dh), 2, 0, 3, 1, 4)
        q, k, v = qkv[0], qkv[1], qkv[2]
        scores = jnp.einsum("bhqd,bhkd->bhqk", q, k) * (Dh ** -0.5)
        p = _softmax(scores, axis=-1)
        o = jnp.einsum("bhqk,bhkd->bhqd", p, v)
        return (lambda x, *d: x.transpose(*d))(o, 0, 2, 1, 3).reshape(B, S, D) @ wo

    def _B_ref(x, w1, b1, w2, b2):
        h = jnp.einsum("bsd,df->bsf", x, w1) + b1
        h = _gelu(h)
        return jnp.einsum("bsf,fd->bsd", h, w2) + b2

    x = A_x
    x = x + _A_ref(_layernorm(x, axis=-1), A_wqkv, A_wo)
    x = x + _B_ref(_layernorm(x, axis=-1), B_w1, B_b1, B_w2, B_b2)
    x = x + _A_ref(_layernorm(x, axis=-1), A_wqkv, A_wo)
    x = x + _B_ref(_layernorm(x, axis=-1), B_w1, B_b1, B_w2, B_b2)
    return x
```

```python
import functools
import math

import jax
import jax.numpy as jnp
from jax import lax
import jax.experimental.pallas as pl
import jax.experimental.pallas.tpu as pltpu

F32 = jnp.float32
BF16 = jnp.bfloat16

H = 32
DH = 16
GH = 8
TQ = 512
CK = 128
U = 4
TS = 256
EPS = 1e-5
NT_DIMS = (((1,), (1,)), ((), ()))


def _layernorm_bf16(x):
    m = jnp.mean(x, axis=-1, keepdims=True)
    xc = x - m
    v = jnp.mean(xc * xc, axis=-1, keepdims=True)
    return (xc * lax.rsqrt(v + EPS)).astype(BF16)


def _gelu(x):
    c0 = math.sqrt(2.0 / math.pi)
    c1 = c0 * 0.044715
    t = jnp.tanh(x * (c0 + c1 * (x * x)))
    hx = 0.5 * x
    return hx + hx * t


def _kernel(x_ref, wqkv_ref, wo_ref, w1_ref, b1_ref, w2_ref, b2_ref, o_ref,
            xr_ref, wqvt_ref, k_ref, qt_ref, vt_ref, ot_ref, s_ref, m_ref,
            *, S, D):
    NQ = S // TQ
    NU = NQ * H
    NC = S // CK
    R = CK // 8
    NB = NU // U
    NG = D // 128
    qscale = (DH ** -0.5) * math.log2(math.e)

    wqvt_ref[0:D, :] = wqkv_ref[:, 0:D].astype(F32).T.astype(BF16)
    wqvt_ref[D:2 * D, :] = wqkv_ref[:, 2 * D:3 * D].astype(F32).T.astype(BF16)

    def qkv_tile(i, sub, x):
        xn = _layernorm_bf16(x)
        rows = pl.ds(pl.multiple_of(i * TQ + sub * TS, TS), TS)
        k = jnp.dot(xn, wqkv_ref[:, D:2 * D], preferred_element_type=F32).astype(BF16)
        for g in range(NG):
            k_ref[g, rows, :] = k[:, g * 128:(g + 1) * 128]
        qvt = lax.dot_general(wqvt_ref[...], xn, NT_DIMS, preferred_element_type=F32)
        qt = (qvt[0:D] * qscale).astype(BF16)
        for g in range(NG):
            qt_ref[i * NG + g, :, sub * TS:(sub + 1) * TS] = qt[g * 128:(g + 1) * 128]
        vt_ref[i, :, :, sub * TS:(sub + 1) * TS] = (
            qvt[D:2 * D].astype(BF16).reshape(H, DH, TS))

    def first_tile(i, carry):
        for sub in range(TQ // TS):
            rows = pl.ds(pl.multiple_of(i * TQ + sub * TS, TS), TS)
            x = x_ref[rows, :].astype(F32)
            xr_ref[rows, :] = x
            qkv_tile(i, sub, x)
        return carry

    lax.fori_loop(0, NQ, first_tile, 0)

    neg = jnp.full((8, TQ), -jnp.inf, F32)

    def masked_qt(u):
        ig = lax.shift_right_logical(u, 3)
        w = pltpu.bitcast(qt_ref[ig], jnp.uint32)
        row = lax.broadcasted_iota(jnp.int32, w.shape, 0)
        w = jnp.where(lax.shift_right_logical(row, 3) == (u & (GH - 1)), w, jnp.uint32(0))
        return ig & (NG - 1), pltpu.bitcast(w, BF16)

    def unit(a, uq, up):
        if uq is not None:
            g, qm = masked_qt(uq)
            mx = neg
        if up is not None:
            h = up & (H - 1)
            mb = m_ref[a]
            acc = jnp.zeros((DH, TQ), F32)
            l = jnp.zeros((8, TQ), F32)
        for c in range(NC):
            sl = pl.ds(c * CK, CK)
            if uq is not None:
                s = jnp.dot(k_ref[g, sl, :], qm, preferred_element_type=F32)
            if up is not None:
                p = jnp.exp2(s_ref[a, sl, :].reshape(R, 8, TQ) - mb[None])
            if uq is not None:
                s_ref[a, sl, :] = s
                mx = jnp.maximum(mx, jnp.max(s.reshape(R, 8, TQ), axis=0))
            if up is not None:
                for r in range(R - 1, -1, -2):
                    l = l + (p[r] + p[r - 1])
                off = (c * CK) % TQ
                v = vt_ref[(c * CK) // TQ, h, :, off:off + CK]
                acc = acc + jnp.dot(v, p.reshape(CK, TQ).astype(BF16),
                                    preferred_element_type=F32)
        if up is not None:
            ls = jnp.sum(l, axis=0, keepdims=True)
            ot_ref[up] = acc * pl.reciprocal(ls, approx=False)
        if uq is not None:
            m_ref[a] = jnp.broadcast_to(jnp.max(mx, axis=0, keepdims=True), (8, TQ))

    def attention():
        for a in range(U):
            unit(a, a, None)

        def block(t, carry):
            for a in range(U):
                unit(a, t * U + a, (t - 1) * U + a)
            return carry

        lax.fori_loop(1, NB, block, 0)
        for a in range(U):
            unit(a, None, (NB - 1) * U + a)

    def post_tile(i, last):
        for sub in range(TQ // TS):
            rows = pl.ds(pl.multiple_of(i * TQ + sub * TS, TS), TS)
            ot = ot_ref[pl.ds(pl.multiple_of(i * H, H), H), :, sub * TS:(sub + 1) * TS]
            o = ot.reshape(D, TS).T.astype(BF16)
            x1 = xr_ref[rows, :] + jnp.dot(o, wo_ref[...], preferred_element_type=F32)
            xn = _layernorm_bf16(x1)
            hh = jnp.dot(xn, w1_ref[...], preferred_element_type=F32) + b1_ref[...]
            hh = _gelu(hh).astype(BF16)
            x2 = x1 + (jnp.dot(hh, w2_ref[...], preferred_element_type=F32) + b2_ref[...])
            if last:
                o_ref[rows, :] = x2.astype(o_ref.dtype)
            else:
                xr_ref[rows, :] = x2
                qkv_tile(i, sub, x2)

    def post(last):
        def body(i, carry):
            post_tile(i, last)
            return carry
        lax.fori_loop(0, NQ, body, 0)

    attention()
    post(False)
    attention()
    post(True)


@jax.jit
def pallas_interleave_layers__mha_block__dense_activation_gelu__prompt_kernel(
    A_x: jax.Array,
    A_wqkv: jax.Array,
    A_wo: jax.Array,
    B_x: jax.Array,
    B_w1: jax.Array,
    B_b1: jax.Array,
    B_w2: jax.Array,
    B_b2: jax.Array,
):
    B, S, D = A_x.shape
    FF = B_w1.shape[1]
    NQ = S // TQ
    x = A_x.reshape(S, D)
    b1 = B_b1.reshape(1, FF).astype(F32)
    b2 = B_b2.reshape(1, D).astype(F32)

    out = pl.pallas_call(
        functools.partial(_kernel, S=S, D=D),
        out_shape=jax.ShapeDtypeStruct((S, D), A_x.dtype),
        scratch_shapes=[
            pltpu.VMEM((S, D), F32),
            pltpu.VMEM((2 * D, D), BF16),
            pltpu.VMEM((D // 128, S, 128), BF16),
            pltpu.VMEM((NQ * (D // 128), 128, TQ), BF16),
            pltpu.VMEM((NQ, H, DH, TQ), BF16),
            pltpu.VMEM((NQ * H, DH, TQ), F32),
            pltpu.VMEM((U, S, TQ), F32),
            pltpu.VMEM((U, 8, TQ), F32),
        ],
        compiler_params=pltpu.CompilerParams(vmem_limit_bytes=100 * 1024 * 1024),
    )(x, A_wqkv, A_wo, B_w1, b1, B_w2, b2)
    return out.reshape(B, S, D)
```

```python
import functools
import math

import jax
import jax.numpy as jnp
from jax import lax
import jax.experimental.pallas as pl
import jax.experimental.pallas.tpu as pltpu

F32 = jnp.float32
BF16 = jnp.bfloat16
U32 = jnp.uint32

H = 32
DH = 16
GH = 8
TQ = 512
TS = 256
NL = TQ // 128
EPS = 1e-5
SK = 3
VLEAD = -4
KBAR_ROWS = 64
L_SAFE = 2.0 ** 40
NT_DIMS = (((1,), (1,)), ((), ()))


def _layernorm_bf16(x):
    m = jnp.mean(x, axis=-1, keepdims=True)
    xc = x - m
    v = jnp.mean(xc * xc, axis=-1, keepdims=True)
    return (xc * lax.rsqrt(v + EPS)).astype(BF16)


def _gelu(x):
    c0 = math.sqrt(2.0 / math.pi)
    c1 = c0 * 0.044715
    t = jnp.tanh(x * (c0 + c1 * (x * x)))
    hx = 0.5 * x
    return hx + hx * t


def _pack(x):
    return pltpu.bitcast(x.astype(BF16), U32)


def _unpack(w):
    return pltpu.bitcast(w, BF16)


def _kernel(x_ref, wqkv_ref, wo_ref, w1_ref, b1_ref, w2_ref, b2_ref, o_ref,
            xr_ref, xn_ref, wk_ref, wqvt_ref, k_ref, qt_ref, vt_ref, qf_ref, kb_ref,
            ot_ref, s_ref,
            *, S, D):
    NQ = S // TQ
    NU = NQ * H
    NT = S // 128
    NG = D // 128
    NB = NQ * NG
    NSUB = TQ // TS
    qscale = (DH ** -0.5) * math.log2(math.e)

    def rows_of(i, sub):
        return pl.ds(pl.multiple_of(i * TQ + sub * TS, TS), TS)

    for g in range(NG):
        wk_ref[g] = wqkv_ref[:, D + g * 128:D + (g + 1) * 128]
        wqvt_ref[g, 0:128, :] = (
            wqkv_ref[:, g * 128:(g + 1) * 128].astype(F32).T.astype(BF16))
        wqvt_ref[g, 128:256, :] = (
            wqkv_ref[:, 2 * D + g * 128:2 * D + (g + 1) * 128].astype(F32).T.astype(BF16))

    def init_tile(i, carry):
        for sub in range(NSUB):
            x = x_ref[rows_of(i, sub), :].astype(F32)
            xr_ref[rows_of(i, sub), :] = x
            xn_ref[rows_of(i, sub), :] = _layernorm_bf16(x)
        return carry

    lax.fori_loop(0, NQ, init_tile, 0)

    def qkv_group(g, carry):
        xv = jnp.concatenate(
            [xn_ref[a * 128 + 112:a * 128 + 128, :] for a in range(NT)], axis=0)
        k = jnp.dot(xv, wk_ref[g], preferred_element_type=F32)
        kbar = jnp.mean(k[0:KBAR_ROWS], axis=0, keepdims=True)
        k = k - kbar
        kp = _pack(k)
        for a in range(NT):
            k_ref[g, a * 64 + 56:a * 64 + 64, :] = kp[a * 8:(a + 1) * 8]
        kr = pltpu.bitcast(k.astype(BF16).astype(F32), U32).reshape(NT, 16, 128)
        src = kr[:, 8:16] | lax.shift_right_logical(kr[:, 0:8], jnp.uint32(16))
        src = src.reshape(NT * 8, 128)
        for lane in range(128):
            col = jnp.broadcast_to(src[:, lane:lane + 1], (NT * 8, 128))
            lo = pltpu.bitcast(lax.shift_left(col, jnp.uint32(16)), F32)
            hi = pltpu.bitcast(col & jnp.uint32(0xFFFF0000), F32)
            kb_ref[g, lane // DH, :, lane % DH, 0] = lo.reshape(NT, 8, 128)
            kb_ref[g, lane // DH, :, lane % DH, 1] = hi.reshape(NT, 8, 128)
        for i in range(NQ):
            tiles = range(i * NL, (i + 1) * NL)
            xm = jnp.concatenate(
                [xn_ref[a * 128:a * 128 + 112, :] for a in tiles], axis=0)
            kp = _pack(jnp.dot(xm, wk_ref[g], preferred_element_type=F32) - kbar)
            for n, a in enumerate(tiles):
                k_ref[g, a * 64:a * 64 + 56, :] = kp[n * 56:(n + 1) * 56]
        for i in range(NQ):
            qvt = lax.dot_general(wqvt_ref[g], xn_ref[i * TQ:(i + 1) * TQ, :], NT_DIMS,
                                  preferred_element_type=F32)
            qt = qvt[0:128] * qscale
            qt_ref[g * NQ + i] = _pack(qt)
            vp = _pack(qvt[128:256])
            for a in range(NL):
                qf_ref[g * NQ + i, a] = qt[:, a * 128:(a + 1) * 128]
                vt_ref[g, i * NL + a] = vp[:, a * 128:(a + 1) * 128]
        return carry

    def post_tile(i, carry):
        subs = range(NSUB)
        x1 = []
        for sub in subs:
            ot = ot_ref[pl.ds(pl.multiple_of(i * H, H), H), :, sub * TS:(sub + 1) * TS]
            o = ot.reshape(D, TS).T.astype(BF16)
            x1.append(jnp.dot(o, wo_ref[...], preferred_element_type=F32)
                      + xr_ref[rows_of(i, sub), :])
        hh = []
        for sub in subs:
            xn = _layernorm_bf16(x1[sub])
            h = jnp.dot(xn, w1_ref[...], preferred_element_type=F32) + b1_ref[...]
            hh.append(_gelu(h).astype(BF16))
        for sub in subs:
            x2 = (jnp.dot(hh[sub], w2_ref[...], preferred_element_type=F32)
                  + (x1[sub] + b2_ref[...]))
            o_ref[rows_of(i, sub), :] = x2.astype(o_ref.dtype)
            xr_ref[rows_of(i, sub), :] = x2
            xn_ref[rows_of(i, sub), :] = _layernorm_bf16(x2)
        return carry

    zacc = jnp.zeros((DH, TQ), F32)
    zl = jnp.zeros((8, TQ), F32)

    def finish(slot, acc, l):
        ls = jnp.sum(l, axis=0, keepdims=True)
        ot_ref[slot] = acc * pl.reciprocal(ls, approx=False)
        return ls

    M = [(k, r) for k in range(NT) for r in range(6, -1, -1)]
    bounds = [0] + [7 * k - SK for k in range(1, NT + 1)] + [7 * NT]
    steps = [list(range(a, b)) for a, b in zip(bounds[:-1], bounds[1:])]
    NPEND = 2

    def fast_block(t, carry):
        acc, lprev, lmax, pend = carry
        g = lax.shift_right_logical(t, 2)
        i = t & (NQ - 1)
        tp = jnp.maximum(t - 1, 0)
        gprev = lax.shift_right_logical(tp, 2)
        slot_prev = jnp.where(t == 0, NU, (tp & (NQ - 1)) * H + gprev * GH + (GH - 1))
        never = lax.broadcasted_iota(jnp.int32, (8, 128), 0) > (t + 8)

        queue = [[n, -1, NT - NPEND + n, pend[n]] for n in range(NPEND)]
        lsum = {-1: lprev}
        pb = {}
        pops = []
        clock = 0
        gs = 0
        uniq = 0

        def consume(j, k, r, top, bot):
            pt = jnp.exp2(top)
            pm = jnp.exp2(bot)
            lsum[j] = lsum[j] + (pt + pm)
            pb[(k, r)] = [pt, pm]

        for j in range(GH):
            parts = []
            if j > 0:
                parts.append(jnp.zeros((16 * j, TQ), BF16))
            parts.append(_unpack(qt_ref[t, 8 * j:8 * j + 8, :]))
            if j < GH - 1:
                parts.append(jnp.zeros((16 * (GH - 1 - j), TQ), BF16))
            qm = jnp.concatenate(parts, axis=0)
            lsum[j] = zl
            for si, st in enumerate(steps):
                lhs = _unpack(jnp.concatenate(
                    [k_ref[g, pl.ds(M[n][0] * 64 + M[n][1] * 8, 8), :] for n in st], axis=0))
                s = jnp.dot(lhs, qm, preferred_element_type=F32)
                for b, n in enumerate(st):
                    k, r = M[n]
                    if r == 6:
                        res = {}
                        for lt in range(NL):
                            want = clock - VLEAD * 8 - 128 + lt * 32
                            cand = [pp for pp in pops if pp[0] <= want]
                            rel = cand[-1][1] if cand else None
                            uniq += 1
                            tq = jnp.minimum(t, 1000 + uniq)
                            gq = lax.shift_right_logical(tq, 2)
                            for d in range(DH):
                                qd = qf_ref[tq, lt, pl.ds(j * DH + d, 8, stride=0), :]
                                for kg in range(2):
                                    tt = kb_ref[gq, j, k, d, kg] * qd
                                    if d > 0:
                                        res[kg, lt] = res[kg, lt] + tt
                                    elif rel is None:
                                        res[kg, lt] = tt
                                    else:
                                        res[kg, lt] = jnp.where(never, rel, tt)
                        top, bot = [jnp.concatenate([res[kg, lt] for lt in range(NL)], axis=1)
                                    for kg in range(2)]
                        consume(j, k, 7, top, bot)
                    blk = s[b * 16:(b + 1) * 16]
                    pops.append((clock, blk[0:8, 0:128]))
                    pops.append((clock + 8, blk[8:16, 0:128]))
                    pops = pops[-64:]
                    clock += 16
                    consume(j, k, r, blk[0:8], blk[8:16])
                    if r == 0:
                        p = jnp.concatenate(
                            sum([pb.pop((k, rr)) for rr in range(8)], []), axis=0).astype(BF16)
                        queue.append([gs + 1, j, k, p])
                if si < len(steps) - 1:
                    e = [e for e in queue if e[0] <= gs][0]
                    queue.remove(e)
                    _, ja, k, p = e
                    ga, jj = (gprev, GH - 1) if ja < 0 else (g, ja)
                    v = _unpack(vt_ref[ga, k, jj * 8:(jj + 1) * 8, :])
                    acc = jnp.dot(v, p, preferred_element_type=F32) + acc
                    pops.append((clock, acc[0:8, 0:128]))
                    pops.append((clock + 8, acc[8:16, 0:128]))
                    clock += 16
                    if k == NT - 1:
                        slot = slot_prev if ja < 0 else i * H + g * GH + ja
                        lmax = jnp.maximum(lmax, finish(slot, acc, lsum[ja]))
                        acc = zacc
                    gs += 1
        assert len(queue) == NPEND and all(e[1] == GH - 1 for e in queue)
        return acc, lsum[GH - 1], lmax, [e[3] for e in queue]

    def exact_unit(u, carry):
        i = lax.shift_right_logical(u, 5)
        h = u & (H - 1)
        g = lax.shift_right_logical(h, 3)
        j = h & (GH - 1)
        w = qt_ref[g * NQ + i]
        row = lax.broadcasted_iota(jnp.int32, w.shape, 0)
        w = jnp.where(lax.shift_right_logical(row, 3) == j, w, jnp.uint32(0))
        s_ref[...] = jnp.dot(_unpack(k_ref[g]), _unpack(w), preferred_element_type=F32)
        m = jnp.max(s_ref[...], axis=0, keepdims=True)
        acc = zacc
        l = zl
        for k in range(NT):
            p = jnp.exp2(s_ref[k * 128:(k + 1) * 128, :] - m)
            l = l + jnp.sum(p.reshape(16, 8, TQ), axis=0)
            v = _unpack(vt_ref[g, k, pl.ds(pl.multiple_of(j * 8, 8), 8), :])
            acc = jnp.dot(v, p.astype(BF16), preferred_element_type=F32) + acc
        finish(u, acc, l)
        return carry

    pend_tiles = list(range(NT - NPEND, NT))

    def attention():
        init = (zacc, jnp.ones((8, TQ), F32), jnp.zeros((1, TQ), F32),
                [jnp.zeros((128, TQ), BF16)] * len(pend_tiles))
        acc, l, lmax, pend = lax.fori_loop(0, NB, fast_block, init)
        for k, p in zip(pend_tiles, pend):
            v = _unpack(vt_ref[NG - 1, k, (GH - 1) * 8:GH * 8, :])
            acc = jnp.dot(v, p, preferred_element_type=F32) + acc
        lmax = jnp.maximum(lmax, finish(NU - 1, acc, l))
        unsafe = jnp.max(jnp.where(lmax <= L_SAFE, 0, 1))

        @pl.when(unsafe > 0)
        def _():
            lax.fori_loop(0, NU, exact_unit, 0)

    def layer(n, carry):
        lax.fori_loop(0, NG, qkv_group, 0)
        attention()
        lax.fori_loop(0, NQ, post_tile, 0)
        return carry

    lax.fori_loop(0, 2, layer, 0)


@jax.jit
def pallas_interleave_layers__mha_block__dense_activation_gelu__prompt_kernel(
    A_x: jax.Array,
    A_wqkv: jax.Array,
    A_wo: jax.Array,
    B_x: jax.Array,
    B_w1: jax.Array,
    B_b1: jax.Array,
    B_w2: jax.Array,
    B_b2: jax.Array,
):
    B, S, D = A_x.shape
    FF = B_w1.shape[1]
    NQ = S // TQ
    NT = S // 128
    NG = D // 128
    x = A_x.reshape(S, D)
    b1 = B_b1.reshape(1, FF).astype(F32)
    b2 = B_b2.reshape(1, D).astype(F32)

    out = pl.pallas_call(
        functools.partial(_kernel, S=S, D=D),
        out_shape=jax.ShapeDtypeStruct((S, D), A_x.dtype),
        scratch_shapes=[
            pltpu.VMEM((S, D), F32),
            pltpu.VMEM((S, D), BF16),
            pltpu.VMEM((NG, D, 128), BF16),
            pltpu.VMEM((NG, 256, D), BF16),
            pltpu.VMEM((NG, S // 2, 128), U32),
            pltpu.VMEM((NG * NQ, 64, TQ), U32),
            pltpu.VMEM((NG, NT, 64, 128), U32),
            pltpu.VMEM((NG * NQ, NL, 128, 128), F32),
            pltpu.VMEM((NG, GH, NT, DH, 2, 8, 128), F32),
            pltpu.VMEM((NQ * H + 1, DH, TQ), F32),
            pltpu.VMEM((S, TQ), F32),
        ],
        compiler_params=pltpu.CompilerParams(vmem_limit_bytes=120 * 1024 * 1024),
    )(x, A_wqkv, A_wo, B_w1, b1, B_w2, b2)
    return out.reshape(B, S, D)
```

```python
import functools
import math

import jax
import jax.numpy as jnp
from jax import lax
import jax.experimental.pallas as pl
import jax.experimental.pallas.tpu as pltpu

F32 = jnp.float32
BF16 = jnp.bfloat16
U32 = jnp.uint32

H = 32
DH = 16
GH = 8
TQ = 512
TS = 256
NL = TQ // 128
EPS = 1e-5
SK = 4
VLEAD = -4
NVB = 16
VPH = 4
KBAR_ROWS = 64
L_SAFE = 2.0 ** 40
NT_DIMS = (((1,), (1,)), ((), ()))


def _layernorm_bf16(x):
    m = jnp.mean(x, axis=-1, keepdims=True)
    xc = x - m
    v = jnp.mean(xc * xc, axis=-1, keepdims=True)
    return (xc * lax.rsqrt(v + EPS)).astype(BF16)


def _gelu(x):
    c0 = math.sqrt(2.0 / math.pi)
    c1 = c0 * 0.044715
    t = jnp.tanh(x * (c0 + c1 * (x * x)))
    hx = 0.5 * x
    return hx + hx * t


def _pack(x):
    return pltpu.bitcast(x.astype(BF16), U32)


def _unpack(w):
    return pltpu.bitcast(w, BF16)


def _kernel(x_hbm, wqkv_hbm, wo_hbm, w1_hbm, b1_hbm, w2_hbm, b2_hbm, o_hbm,
            x_ref, wqv_ref, wo_ref, w1_ref, w2_ref, o_ref,
            xr_ref, xn_ref, wk_ref, wqvt_ref, k_ref, qt_ref, vt_ref, qf_ref, kb_ref,
            ot_ref, l_ref, ob_ref, xl_ref, p_ref, s_ref, b1_ref, b2_ref, sem_x, sem_g, sem_w, sem_o,
            *, S, D):
    NQ = S // TQ
    NU = NQ * H
    NT = S // 128
    NG = D // 128
    NB = NQ * NG
    NSUB = TQ // TS
    qscale = (DH ** -0.5) * math.log2(math.e)
    G = [(k, r) for k in range(NT) for r in range(7, -1, -1)]
    vpos = [VPH + (n * len(G)) // NVB for n in range(NVB)]
    VB = [G[n] for n in vpos]
    M = [b for b in G if b not in VB]

    def rows_of(i, sub):
        return pl.ds(pl.multiple_of(i * TQ + sub * TS, TS), TS)

    def x_copy(i):
        rows = pl.ds(pl.multiple_of(i * TS, TS), TS)
        return pltpu.make_async_copy(x_hbm.at[rows, :], x_ref.at[rows, :], sem_x.at[i])

    def o_copy(i):
        rows = pl.ds(pl.multiple_of(i * TS, TS), TS)
        return pltpu.make_async_copy(o_ref.at[rows, :], o_hbm.at[rows, :], sem_o.at[i])

    w_copies = [
        pltpu.make_async_copy(src, dst, sem_w.at[n])
        for n, (src, dst) in enumerate(
            [(wo_hbm, wo_ref), (w1_hbm, w1_ref), (w2_hbm, w2_ref),
             (b1_hbm, b1_ref), (b2_hbm, b2_ref)])
    ]

    def g_copy(g, n):
        dst = wk_ref.at[g] if n == 0 else wqv_ref.at[g, n - 1]
        col = pl.multiple_of((D, 0, 2 * D)[n] + g * 128, 128)
        return pltpu.make_async_copy(
            wqkv_hbm.at[:, pl.ds(col, 128)], dst, sem_g.at[g * 3 + n])

    def init_rows(i, carry):
        x_copy(i).wait()
        rows = pl.ds(pl.multiple_of(i * TS, TS), TS)
        x = x_ref[rows, :].astype(F32)
        xr_ref[rows, :] = x
        xn_ref[rows, :] = _layernorm_bf16(x)
        return carry

    def start_group(g):
        for n in range(3):
            g_copy(g, n).start()

    for i in range(S // TS):
        x_copy(i).start()
    start_group(0)
    xl_ref[...] = jnp.zeros(xl_ref.shape, F32)
    p_ref[...] = jnp.zeros(p_ref.shape, F32)
    lax.fori_loop(0, S // TS, init_rows, 0)
    for g in range(1, NG):
        start_group(g)
    for c in w_copies:
        c.start()

    def qkv_group(first, g, carry):
        if first:
            for n in range(3):
                g_copy(g, n).wait()
            for n in range(2):
                wqvt_ref[g, n * 128:(n + 1) * 128, :] = (
                    wqv_ref[g, n].astype(F32).T.astype(BF16))
        xv = jnp.concatenate(
            [xn_ref[k * 128 + r * 16:k * 128 + r * 16 + 16, :] for k, r in VB], axis=0)
        kv = jnp.dot(xv, wk_ref[g], preferred_element_type=F32)
        kbar = jnp.mean(kv[0:KBAR_ROWS], axis=0, keepdims=True)
        kv = kv - kbar
        kp = _pack(kv)
        for n, (k, r) in enumerate(VB):
            k_ref[g, k * 64 + r * 8:k * 64 + r * 8 + 8, :] = kp[n * 8:(n + 1) * 8]
        kr = pltpu.bitcast(kv.astype(BF16).astype(F32), U32).reshape(NVB, 16, 128)
        src = kr[:, 8:16] | lax.shift_right_logical(kr[:, 0:8], jnp.uint32(16))
        src = src.reshape(NVB * 8, 128)
        for lane in range(128):
            col = jnp.broadcast_to(src[:, lane:lane + 1], (NVB * 8, 128))
            lo = pltpu.bitcast(lax.shift_left(col, jnp.uint32(16)), F32)
            hi = pltpu.bitcast(col & jnp.uint32(0xFFFF0000), F32)
            kb_ref[g, lane // DH, :, lane % DH, 0] = lo.reshape(NVB, 8, 128)
            kb_ref[g, lane // DH, :, lane % DH, 1] = hi.reshape(NVB, 8, 128)
        for i in range(NQ):
            blocks = sorted(b for b in M if b[0] // NL == i)
            xm = jnp.concatenate(
                [xn_ref[k * 128 + r * 16:k * 128 + r * 16 + 16, :] for k, r in blocks], axis=0)
            km = jnp.dot(xm, wk_ref[g], preferred_element_type=F32) - kbar
            kp = _pack(km)
            for n, (k, r) in enumerate(blocks):
                k_ref[g, k * 64 + r * 8:k * 64 + r * 8 + 8, :] = kp[n * 8:(n + 1) * 8]
        for i in range(NQ):
            qvt = lax.dot_general(wqvt_ref[g], xn_ref[i * TQ:(i + 1) * TQ, :], NT_DIMS,
                                  preferred_element_type=F32)
            qt = qvt[0:128] * qscale
            qt_ref[g * NQ + i] = _pack(qt)
            vp = _pack(qvt[128:256])
            for a in range(NL):
                qf_ref[g * NQ + i, a] = qt[:, a * 128:(a + 1) * 128]
                vt_ref[g, i * NL + a] = vp[:, a * 128:(a + 1) * 128]
        return carry

    def norm_cols(i, c, rel=None, store=True):
        units = pl.ds(pl.multiple_of(i * H, H), H)
        cols = slice(c * 128, (c + 1) * 128)
        l = l_ref[units, :, cols]
        if rel is not None:
            l = rel(l)
        ls = jnp.sum(l, axis=1, keepdims=True)
        r = pl.reciprocal(ls, approx=True)
        r = r * (2.0 - ls * r)
        ot = ot_ref[units, :, cols] * r
        o = ot.reshape(D, 128).T
        if not store:
            return o
        ob_ref[c * 128:(c + 1) * 128, :] = o.astype(BF16)

    def ln_last(i, rel=None):
        x = xl_ref[...]
        if rel is not None:
            x = jnp.concatenate([rel(x[:, 0:128]), x[:, 128:]], axis=1)
        xn_ref[rows_of(i, NSUB - 1), :] = _layernorm_bf16(x)

    def post_tile(i, carry):
        subs = range(NSUB)
        b1 = b1_ref[...].astype(F32)
        b2 = b2_ref[...].astype(F32)
        x1 = []
        for sub in subs:
            if sub == 0:
                o = ob_ref[...]
            else:
                o = jnp.concatenate([norm_cols(i, c, store=False)
                                     for c in range(NL // 2, NL)], axis=0).astype(BF16)
            x1.append(jnp.dot(o, wo_ref[...], preferred_element_type=F32)
                      + xr_ref[rows_of(i, sub), :])
        hh = []
        for sub in subs:
            xn = _layernorm_bf16(x1[sub])
            h = jnp.dot(xn, w1_ref[...], preferred_element_type=F32) + b1
            hh.append(_gelu(h).astype(BF16))
        x2 = [jnp.dot(hh[sub], w2_ref[...], preferred_element_type=F32) + (x1[sub] + b2)
              for sub in subs]

        def after(sub, c):
            def rel(v):
                never = lax.broadcasted_iota(jnp.int32, v.shape, 0) > (i + TS)
                return jnp.where(
                    never, x2[sub][:, c * 128:(c + 1) * 128].reshape(v.shape), v)
            return rel

        ln_last(jnp.maximum(i - 1, 0), after(0, 0))
        inext = jnp.minimum(i + 1, NQ - 1)
        for c, (sub, cc) in enumerate([(0, 1), (0, 2)]):
            norm_cols(inext, c, after(sub, cc))
        for sub in subs:
            o_ref[rows_of(i, sub), :] = x2[sub].astype(o_ref.dtype)
            o_copy(i * NSUB + sub).start()
            xr_ref[rows_of(i, sub), :] = x2[sub]
            if sub < NSUB - 1:
                xn_ref[rows_of(i, sub), :] = _layernorm_bf16(x2[sub])
            else:
                xl_ref[...] = x2[sub]
        return carry

    zacc = jnp.zeros((DH, TQ), F32)
    zl = jnp.zeros((8, TQ), F32)

    def finish(slot, acc, l):
        ot_ref[slot] = acc
        l_ref[slot] = l

    ends = [sum(1 for b in M if b[0] <= k) for k in range(NT)]
    bounds = [0] + [e - SK for e in ends] + [len(M)]
    steps = [list(range(a, b)) for a, b in zip(bounds[:-1], bounds[1:])]
    unit_cycles = 16 * (len(M) + NT)
    vat = [p - n for n, p in enumerate(vpos)]
    vclock = [16 * (a + sum(1 for e in bounds[1:-1] if e <= a)) for a in vat]
    voff = min(vclock[n] - ((n * NL + NL - 1) * unit_cycles) // (NVB * NL)
               for n in range(NVB)) - 32 - VLEAD * 8
    NPEND = 2

    def fast_block(t, carry):
        acc, lprev, lmax = carry
        g = lax.shift_right_logical(t, 2)
        i = t & (NQ - 1)
        tp = jnp.maximum(t - 1, 0)
        gprev = lax.shift_right_logical(tp, 2)
        slot_prev = jnp.where(t == 0, NU, (tp & (NQ - 1)) * H + gprev * GH + (GH - 1))
        never = lax.broadcasted_iota(jnp.int32, (8, 128), 0) > (t + 8)

        queue = [[-1, NT - NPEND + n, p_ref[n]] for n in range(NPEND)]
        lsum = {-1: lprev}
        pb = {}
        pops = []
        clock = 0
        uniq = 0

        def consume(j, k, r, top, bot):
            pt = jnp.exp2(top)
            pm = jnp.exp2(bot)
            both = pt + pm
            lsum[j] = both if lsum[j] is None else lsum[j] + both
            pb[(k, r)] = [pt, pm]
            if r == 0:
                p = jnp.concatenate(
                    sum([pb.pop((k, rr)) for rr in range(8)], []), axis=0)
                queue.append([j, k, p])

        for j in range(GH):
            parts = []
            if j > 0:
                parts.append(jnp.zeros((16 * j, TQ), BF16))
            parts.append(_unpack(qt_ref[t, 8 * j:8 * j + 8, :]))
            if j < GH - 1:
                parts.append(jnp.zeros((16 * (GH - 1 - j), TQ), BF16))
            qm = jnp.concatenate(parts, axis=0)
            lsum[j] = None
            t0 = clock
            for si, st in enumerate(steps):
                lhs = _unpack(jnp.concatenate(
                    [k_ref[g, pl.ds(M[n][0] * 64 + M[n][1] * 8, 8), :] for n in st], axis=0))
                s = jnp.dot(lhs, qm, preferred_element_type=F32)
                for b, n in enumerate(st):
                    k, r = M[n]
                    for vn in [vn for vn in range(NVB) if vat[vn] == n]:
                        res = {}
                        for lt in range(NL):
                            want = t0 + voff + ((vn * NL + lt) * unit_cycles) // (NVB * NL)
                            cand = [pp for pp in pops if pp[0] <= want]
                            uniq += 1
                            tq = jnp.minimum(t, 1000 + uniq)
                            gq = lax.shift_right_logical(tq, 2)
                            for d in range(DH):
                                qd = qf_ref[tq, lt, pl.ds(j * DH + d, 8, stride=0), :]
                                if d == 0 and cand:
                                    qd = jnp.where(never, cand[-1][1], qd)
                                for kg in range(2):
                                    tt = kb_ref[gq, j, vn, d, kg] * qd
                                    res[kg, lt] = tt if d == 0 else res[kg, lt] + tt
                        top, bot = [jnp.concatenate([res[kg, lt] for lt in range(NL)], axis=1)
                                    for kg in range(2)]
                        consume(j, VB[vn][0], VB[vn][1], top, bot)
                    blk = s[b * 16:(b + 1) * 16]
                    pops.append((clock, blk[0:8, 0:128]))
                    pops.append((clock + 8, blk[8:16, 0:128]))
                    pops = pops[-64:]
                    clock += 16
                    consume(j, k, r, blk[0:8], blk[8:16])
                if si < len(steps) - 1:
                    ja, k, p = queue.pop(0)
                    ga, jj = (gprev, GH - 1) if ja < 0 else (g, ja)
                    v = _unpack(vt_ref[ga, k, jj * 8:(jj + 1) * 8, :])
                    pv = jnp.dot(v, p.astype(BF16), preferred_element_type=F32)
                    acc = pv if acc is None else pv + acc
                    pops.append((clock, acc[0:8, 0:128]))
                    pops.append((clock + 8, acc[8:16, 0:128]))
                    clock += 16
                    if k == NT - 1:
                        slot = slot_prev if ja < 0 else i * H + g * GH + ja
                        finish(slot, acc, lsum[ja])
                        lmax = jnp.maximum(lmax, lsum[ja])
                        acc = None
        assert len(queue) == NPEND and all(e[0] == GH - 1 for e in queue)
        for n in range(NPEND):
            p_ref[n] = queue[n][2]
        return acc, lsum[GH - 1], lmax

    def exact_unit(u, carry):
        i = lax.shift_right_logical(u, 5)
        h = u & (H - 1)
        g = lax.shift_right_logical(h, 3)
        j = h & (GH - 1)
        w = qt_ref[g * NQ + i]
        row = lax.broadcasted_iota(jnp.int32, w.shape, 0)
        w = jnp.where(lax.shift_right_logical(row, 3) == j, w, jnp.uint32(0))
        s_ref[...] = jnp.dot(_unpack(k_ref[g]), _unpack(w), preferred_element_type=F32)
        m = jnp.max(s_ref[...], axis=0, keepdims=True)
        acc = zacc
        l = zl
        for k in range(NT):
            p = jnp.exp2(s_ref[k * 128:(k + 1) * 128, :] - m)
            l = l + jnp.sum(p.reshape(16, 8, TQ), axis=0)
            v = _unpack(vt_ref[g, k, pl.ds(pl.multiple_of(j * 8, 8), 8), :])
            acc = jnp.dot(v, p.astype(BF16), preferred_element_type=F32) + acc
        finish(u, acc, l)
        return carry

    def attention():
        acc, l, lmax = lax.fori_loop(0, NB, fast_block, (zacc, zl, zl))
        for n in range(NPEND):
            v = _unpack(vt_ref[NG - 1, NT - NPEND + n, (GH - 1) * 8:GH * 8, :])
            acc = jnp.dot(v, p_ref[n].astype(BF16), preferred_element_type=F32) + acc
        finish(NU - 1, acc, l)
        lmax = jnp.maximum(lmax, l)
        unsafe = jnp.max(jnp.where(lmax <= L_SAFE, 0, 1))
        for c in range(NL // 2):
            norm_cols(0, c)

        @pl.when(unsafe > 0)
        def _():
            lax.fori_loop(0, NU, exact_unit, 0)
            for c in range(NL // 2):
                norm_cols(0, c)

    lax.fori_loop(0, NG, functools.partial(qkv_group, True), 0)
    for c in w_copies:
        c.wait()

    def layer(n, carry):
        attention()
        lax.fori_loop(0, NQ, post_tile, 0)

        @pl.when(n == 0)
        def _():
            ln_last(NQ - 1)
            lax.fori_loop(0, NG, functools.partial(qkv_group, False), 0)

        for i in range(S // TS):
            o_copy(i).wait()
        return carry

    lax.fori_loop(0, 2, layer, 0)


@jax.jit
def pallas_interleave_layers__mha_block__dense_activation_gelu__prompt_kernel(
    A_x: jax.Array,
    A_wqkv: jax.Array,
    A_wo: jax.Array,
    B_x: jax.Array,
    B_w1: jax.Array,
    B_b1: jax.Array,
    B_w2: jax.Array,
    B_b2: jax.Array,
):
    B, S, D = A_x.shape
    FF = B_w1.shape[1]
    NQ = S // TQ
    NT = S // 128
    NG = D // 128
    x = A_x.reshape(S, D)
    hbm = pl.BlockSpec(memory_space=pl.ANY)

    out = pl.pallas_call(
        functools.partial(_kernel, S=S, D=D),
        out_shape=jax.ShapeDtypeStruct((S, D), A_x.dtype),
        in_specs=[hbm] * 7,
        out_specs=hbm,
        scratch_shapes=[
            pltpu.VMEM((S, D), BF16),
            pltpu.VMEM((NG, 2, D, 128), BF16),
            pltpu.VMEM((D, D), BF16),
            pltpu.VMEM((D, FF), BF16),
            pltpu.VMEM((FF, D), BF16),
            pltpu.VMEM((S, D), BF16),
            pltpu.VMEM((S, D), F32),
            pltpu.VMEM((S, D), BF16),
            pltpu.VMEM((NG, D, 128), BF16),
            pltpu.VMEM((NG, 256, D), BF16),
            pltpu.VMEM((NG, S // 2, 128), U32),
            pltpu.VMEM((NG * NQ, 64, TQ), U32),
            pltpu.VMEM((NG, NT, 64, 128), U32),
            pltpu.VMEM((NG * NQ, NL, 128, 128), F32),
            pltpu.VMEM((NG, GH, NVB, DH, 2, 8, 128), F32),
            pltpu.VMEM((NQ * H + 1, DH, TQ), F32),
            pltpu.VMEM((NQ * H + 1, 8, TQ), F32),
            pltpu.VMEM((TS, D), BF16),
            pltpu.VMEM((TS, D), F32),
            pltpu.VMEM((2, 128, TQ), F32),
            pltpu.VMEM((S, TQ), F32),
            pltpu.VMEM((FF,), BF16),
            pltpu.VMEM((D,), BF16),
            pltpu.SemaphoreType.DMA((S // TS,)),
            pltpu.SemaphoreType.DMA((3 * NG,)),
            pltpu.SemaphoreType.DMA((5,)),
            pltpu.SemaphoreType.DMA((S // TS,)),
        ],
        compiler_params=pltpu.CompilerParams(vmem_limit_bytes=124 * 1024 * 1024),
    )(x, A_wqkv, A_wo, B_w1, B_b1, B_w2, B_b2)
    return out.reshape(B, S, D)
```

```python
import functools
import math

import jax
import jax.numpy as jnp
from jax import lax
import jax.experimental.pallas as pl
import jax.experimental.pallas.tpu as pltpu

F32 = jnp.float32
BF16 = jnp.bfloat16
U32 = jnp.uint32

H = 32
DH = 16
GH = 8
TQ = 512
TS = 256
NL = TQ // 128
BQ = 2
VR = 3
SK = 4
VLEAD = 48
QS0 = 3
QTAIL = 32
NPEND = 2
KBAR_ROWS = 64
L_SAFE = 2.0 ** 64
F32_MAX = 3.0e38
EPS = 1e-5
NT_DIMS = (((1,), (1,)), ((), ()))
MXU_BLOCKS = [r for r in range(7, -1, -1) if r != VR]
NM = len(MXU_BLOCKS)


def _layernorm(x):
    m = jnp.mean(x, axis=-1, keepdims=True)
    xc = x - m
    v = jnp.mean(xc * xc, axis=-1, keepdims=True)
    return (xc * lax.rsqrt(v + EPS)).astype(BF16), v


def _gelu(x):
    c0 = math.sqrt(2.0 / math.pi)
    c1 = c0 * 0.044715
    t = jnp.tanh(x * (c0 + c1 * (x * x)))
    hx = 0.5 * x
    return hx + hx * t


def _pack(x):
    return pltpu.bitcast(x.astype(BF16), U32)


def _unpack(w):
    return pltpu.bitcast(w, BF16)


def _after(idx, y, v):
    never = lax.broadcasted_iota(jnp.int32, v.shape, 0) > (idx + v.shape[0])
    return jnp.where(never, y.reshape(v.shape), v)


def _bcast_rows(x):
    return jnp.stack([jnp.broadcast_to(x[d:d + 1], (8, 128)) for d in range(8)])


def _kernel(x_hbm, wqkv_hbm, wo_hbm, w1_hbm, b1_hbm, w2_hbm, b2_hbm, o_hbm,
            x_ref, wqv_ref, wo_ref, w1_ref, w2_ref, o_ref,
            xr_ref, xn_ref, wk_ref, wqvt_ref, k_ref, qt_ref, vt_ref, kb_ref,
            ot_ref, l_ref, ob_ref, xl_ref, p_ref, s_ref, qb_refs, b1_ref, b2_ref,
            flag_ref, sem_x, sem_g, sem_w, sem_o, *, S, D):
    NQ = S // TQ
    NU = NQ * H
    NT = S // 128
    NG = D // 128
    NB = NQ * NG
    NSUB = TQ // TS
    KV0 = NT * NM * 8
    qscale = (DH ** -0.5) * math.log2(math.e)

    def rows_of(i, sub):
        return pl.ds(pl.multiple_of(i * TQ + sub * TS, TS), TS)

    def x_copy(i):
        rows = pl.ds(pl.multiple_of(i * TS, TS), TS)
        return pltpu.make_async_copy(x_hbm.at[rows, :], x_ref.at[rows, :], sem_x.at[i])

    def o_copy(i):
        rows = pl.ds(pl.multiple_of(i * TS, TS), TS)
        return pltpu.make_async_copy(o_ref.at[rows, :], o_hbm.at[rows, :], sem_o.at[i])

    def g_copy(g, n):
        dst = wk_ref.at[g] if n == 0 else wqv_ref.at[g, n - 1]
        col = pl.multiple_of((D, 0, 2 * D)[n] + g * 128, 128)
        return pltpu.make_async_copy(
            wqkv_hbm.at[:, pl.ds(col, 128)], dst, sem_g.at[g * 3 + n])

    w_copies = [
        pltpu.make_async_copy(src, dst, sem_w.at[n])
        for n, (src, dst) in enumerate(
            [(wo_hbm, wo_ref), (w1_hbm, w1_ref), (w2_hbm, w2_ref),
             (b1_hbm, b1_ref), (b2_hbm, b2_ref)])
    ]

    def init_rows(i, carry):
        x_copy(i).wait()
        rows = pl.ds(pl.multiple_of(i * TS, TS), TS)
        x = x_ref[rows, :].astype(F32)
        xr_ref[0, rows, :] = x
        xn_ref[rows, :] = _layernorm(x)[0]
        return carry

    for i in range(S // TS):
        x_copy(i).start()
    for n in range(3):
        g_copy(0, n).start()
    xl_ref[...] = jnp.zeros(xl_ref.shape, F32)
    p_ref[...] = jnp.zeros(p_ref.shape, F32)
    lax.fori_loop(0, S // TS, init_rows, 0)
    for g in range(1, NG):
        for n in range(3):
            g_copy(g, n).start()
    for c in w_copies:
        c.start()

    def xn_blocks(blocks):
        return jnp.concatenate(
            [xn_ref[k * 128 + r * 16:k * 128 + r * 16 + 16, :] for k, r in blocks], axis=0)

    def qkv_group(first, g, carry):
        if first:
            for n in range(3):
                g_copy(g, n).wait()
            for n in range(2):
                wqvt_ref[g, n * 128:(n + 1) * 128, :] = (
                    wqv_ref[g, n].astype(F32).T.astype(BF16))
        kv = jnp.dot(xn_blocks([(k, VR) for k in range(NT)]), wk_ref[g],
                     preferred_element_type=F32)
        kbar = jnp.mean(kv[0:KBAR_ROWS], axis=0, keepdims=True)
        kv = kv - kbar
        k_ref[g, KV0:KV0 + NT * 8, :] = _pack(kv)
        kr = pltpu.bitcast(kv.astype(BF16).astype(F32), U32).reshape(NT, 16, 128)
        src = kr[:, 8:16] | lax.shift_right_logical(kr[:, 0:8], jnp.uint32(16))
        src = src.reshape(NT * 8, 128)
        for lane in range(128):
            col = jnp.broadcast_to(src[:, lane:lane + 1], (NT * 8, 128))
            lo = pltpu.bitcast(lax.shift_left(col, jnp.uint32(16)), F32)
            hi = pltpu.bitcast(col & jnp.uint32(0xFFFF0000), F32)
            kb_ref[g, lane // DH, :, lane % DH, 0] = lo.reshape(NT, 8, 128)
            kb_ref[g, lane // DH, :, lane % DH, 1] = hi.reshape(NT, 8, 128)
        for i in range(NQ):
            xm = xn_blocks([(k, r) for k in range(i * NL, (i + 1) * NL) for r in MXU_BLOCKS])
            km = jnp.dot(xm, wk_ref[g], preferred_element_type=F32) - kbar
            k_ref[g, i * NL * NM * 8:(i + 1) * NL * NM * 8, :] = _pack(km)
        qvs = []
        for i in range(NQ):
            qvt = lax.dot_general(wqvt_ref[g], xn_ref[i * TQ:(i + 1) * TQ, :], NT_DIMS,
                                  preferred_element_type=F32)
            qp = _pack(qvt[0:128] * qscale)
            vp = _pack(qvt[128:256])
            qvs.append(qvt)
            for a in range(NL):
                qt_ref[g * NQ + i, a] = qp[:, a * 128:(a + 1) * 128]
                vt_ref[g, i * NL + a] = vp[:, a * 128:(a + 1) * 128]
            if i == BQ - 1:
                rows = jnp.concatenate(
                    [_unpack(qt_ref[b, g]).astype(F32) for b in range(BQ)], axis=0)
        pace = [(i, a, r) for i in range(BQ, NQ) for a in range(NL) for r in range(32)]
        pace = pace[:-QTAIL]
        for n in range(BQ * 16):
            i, a, r = pace[(n * len(pace)) // (BQ * 16)]
            y = qvs[i][r * 8:(r + 1) * 8, a * 128:(a + 1) * 128]
            qb_refs[n // 2][0, g, (n % 2) * 8:(n % 2) * 8 + 8] = _bcast_rows(
                _after(g, y, rows[n * 8:(n + 1) * 8]))
        return carry

    def norm_cols(i, c, y=None):
        units = pl.ds(pl.multiple_of(i * H, H), H)
        cols = slice(c * 128, (c + 1) * 128)
        l = l_ref[units, :, cols]
        if y is not None:
            l = _after(i, y, l)
        ls = jnp.sum(l, axis=1, keepdims=True)
        r = pl.reciprocal(ls, approx=True)
        r = r * (2.0 - ls * r)
        r = jnp.where(jnp.maximum(ls, r) <= L_SAFE, r, jnp.nan)
        return (ot_ref[units, :, cols] * r).reshape(D, 128).T

    def norm_next(i, ys):
        for c in range(TS // 128):
            ob_ref[c * 128:(c + 1) * 128, :] = norm_cols(i, c, ys[c]).astype(BF16)

    def ln_last(i, y=None):
        x = xl_ref[...]
        if y is not None:
            x = jnp.concatenate([_after(i, y, x[:, 0:128]), x[:, 128:]], axis=1)
        xn_ref[rows_of(i, NSUB - 1), :] = _layernorm(x)[0]

    def post_tile(n, i, bad):
        b1 = b1_ref[...].astype(F32)
        b2 = b2_ref[...].astype(F32)

        def col(y, c):
            return y[:, c * 128:(c + 1) * 128]

        x1 = []
        for sub in range(NSUB):
            if sub == 0:
                o = ob_ref[...]
            else:
                o = jnp.concatenate(
                    [norm_cols(i, TS // 128 + c, col(x1[0], c)) for c in range(TS // 128)],
                    axis=0).astype(BF16)
            x1.append(jnp.dot(o, wo_ref[...], preferred_element_type=F32)
                      + xr_ref[n, rows_of(i, sub), :])
        hh = []
        for sub in range(NSUB):
            xn, var = _layernorm(x1[sub])
            bad = jnp.maximum(bad, jnp.max(jnp.where(var <= F32_MAX, 0, 1)))
            h = jnp.dot(xn, w1_ref[...], preferred_element_type=F32) + b1
            hh.append(_gelu(h).astype(BF16))
        x2 = [jnp.dot(hh[sub], w2_ref[...], preferred_element_type=F32) + (x1[sub] + b2)
              for sub in range(NSUB)]
        ln_last(jnp.maximum(i - 1, 0), col(x2[0], 0))
        norm_next(jnp.minimum(i + 1, NQ - 1), [col(x2[0], 1), col(x2[0], 2)])
        for sub in range(NSUB):
            o_ref[rows_of(i, sub), :] = x2[sub].astype(o_ref.dtype)
            o_copy(i * NSUB + sub).start()
            xr_ref[1 - n, rows_of(i, sub), :] = x2[sub]
            if sub < NSUB - 1:
                xn_ref[rows_of(i, sub), :] = _layernorm(x2[sub])[0]
            else:
                xl_ref[...] = x2[sub]
        return bad

    zacc = jnp.zeros((DH, TQ), F32)
    zl = jnp.zeros((8, TQ), F32)

    def tile_rows(blocks):
        return jnp.concatenate([blocks[r] for r in range(8)], axis=0)

    def rowsum(p):
        return jnp.sum(p.reshape(p.shape[0] // 8, 8, TQ), axis=0)

    bounds = [0] + [NM * k - SK for k in range(1, NT + 1)] + [NM * NT]
    period = 16 * (NM + 1)
    vat = 7 - VR

    def fast_block(tb, carry):
        acc, lprev = carry
        t = tb * BQ
        g = lax.shift_right_logical(t, 2)
        i = t & (NQ - 1)
        tn = jnp.minimum(t + BQ, NB - BQ)
        tp = jnp.maximum(t - 1, 0)
        gprev = lax.shift_right_logical(tp, 2)
        slot_prev = jnp.where(t == 0, NU, (tp & (NQ - 1)) * H + gprev * GH + (GH - 1))

        queue = [(-1, NT - NPEND + n, p_ref[n]) for n in range(NPEND)]
        lsum = {-1: lprev}
        done = []
        clock = 0
        uniq = 0

        def result_at(when):
            cand = [e for e in done if e[0] <= when]
            if not cand:
                return None
            return cand[-1][1][cand[-1][2]:cand[-1][2] + 8, 0:128]

        def add_l(u, p):
            lsum[u] = p if lsum[u] is None else lsum[u] + p

        def make_qb(u, part, y):
            lt, half = divmod(part, 2)
            j = u % GH
            src = _unpack(qt_ref[tn + u // GH, lt, 8 * j:8 * j + 8, :]).astype(F32)
            qb_refs[u][0, lt, half * 8:half * 8 + 8] = _bcast_rows(
                _after(t, y, src[half * 8:half * 8 + 8]))

        for u in range(BQ * GH):
            hb, j = divmod(u, GH)
            parts = [jnp.zeros((16 * j, TQ), BF16)] if j > 0 else []
            parts.append(_unpack(jnp.concatenate(
                [qt_ref[t + hb, a, 8 * j:8 * j + 8, :] for a in range(NL)], axis=1)))
            if j < GH - 1:
                parts.append(jnp.zeros((16 * (GH - 1 - j), TQ), BF16))
            qm = jnp.concatenate(parts, axis=0)
            lsum[u] = None
            blocks = {}
            for si in range(NT + 1):
                lo, hi = bounds[si], bounds[si + 1]
                s = jnp.dot(_unpack(k_ref[g, lo * 8:hi * 8, :]), qm,
                            preferred_element_type=F32)
                e = jnp.exp2(s)
                for n in range(lo, hi):
                    k, pos = divmod(n, NM)
                    if pos == vat:
                        cols = []
                        for lt in range(NL):
                            uniq += 1
                            tq = jnp.minimum(t, 1000 + uniq)
                            qb = qb_refs[u][tq - t, lt]
                            y = result_at(clock - VLEAD - ((NL - 1 - lt) * period) // NL)
                            if y is not None:
                                qb = jnp.concatenate(
                                    [_after(t, y, qb[0])[None], qb[1:]], axis=0)
                            kb = kb_ref[lax.shift_right_logical(tq, 2), j, k]
                            cols.append(jnp.sum(kb * qb[:, None], axis=0))
                        ev = jnp.exp2(jnp.concatenate(cols, axis=2))
                        add_l(u, ev[0] + ev[1])
                        blocks[VR] = ev.reshape(16, TQ)
                    row = (n - lo) * 16
                    done.append((clock, s, row))
                    done.append((clock + 8, s, row + 8))
                    clock += 16
                    blocks[MXU_BLOCKS[pos]] = e[row:row + 16]
                    add_l(u, e[row:row + 8] + e[row + 8:row + 16])
                    if pos == NM - 1:
                        queue.append((u, k, tile_rows(blocks)))
                        blocks = {}
                done = done[-48:]
                if u > 0 and QS0 <= si < QS0 + 2 * NL:
                    make_qb(u - 1, si - QS0, result_at(clock))
                if si < NT:
                    ua, k, p = queue.pop(0)
                    ga, ja = (gprev, GH - 1) if ua < 0 else (g, ua % GH)
                    v = _unpack(vt_ref[ga, k, ja * 8:(ja + 1) * 8, :])
                    pv = jnp.dot(v, p.astype(BF16), preferred_element_type=F32)
                    acc = pv if acc is None else pv + acc
                    done.append((clock, acc, 0))
                    done.append((clock + 8, acc, 8))
                    clock += 16
                    if k == NT - 1:
                        slot = slot_prev if ua < 0 else (i + ua // GH) * H + g * GH + ja
                        ot_ref[slot] = acc
                        l_ref[slot] = lsum[ua]
                        acc = None
        assert [e[:2] for e in queue] == [
            (BQ * GH - 1, NT - NPEND + n) for n in range(NPEND)]
        for n in range(NPEND):
            p_ref[n] = queue[n][2]
        for part in range(2 * NL):
            make_qb(BQ * GH - 1, part, result_at(clock - 128 + 8 * part))
        return acc, lsum[BQ * GH - 1]

    def exact_unit(u, carry):
        i = lax.shift_right_logical(u, 5)
        h = u & (H - 1)
        g = lax.shift_right_logical(h, 3)
        j = h & (GH - 1)
        w = jnp.concatenate([qt_ref[g * NQ + i, a] for a in range(NL)], axis=1)
        row = lax.broadcasted_iota(jnp.int32, w.shape, 0)
        qm = _unpack(jnp.where(lax.shift_right_logical(row, 3) == j, w, jnp.uint32(0)))

        def score(k, mx):
            kk = jnp.concatenate(
                [k_ref[g, pl.ds(pl.multiple_of(k * (NM * 8), 8), NM * 8), :],
                 k_ref[g, pl.ds(pl.multiple_of(KV0 + k * 8, 8), 8), :]], axis=0)
            sc = jnp.dot(_unpack(kk), qm, preferred_element_type=F32)
            s_ref[k] = tile_rows({r: sc[n * 16:(n + 1) * 16]
                                  for n, r in enumerate(MXU_BLOCKS + [VR])})
            return jnp.maximum(mx, jnp.max(sc.reshape(16, 8, TQ), axis=0))

        mx = lax.fori_loop(0, NT, score, jnp.full((8, TQ), -jnp.inf, F32))
        m = jnp.max(mx, axis=0, keepdims=True)

        def pv(k, st):
            p = jnp.exp2(s_ref[k] - m)
            v = _unpack(vt_ref[g, k, pl.ds(pl.multiple_of(j * 8, 8), 8), :])
            return (jnp.dot(v, p.astype(BF16), preferred_element_type=F32) + st[0],
                    st[1] + rowsum(p))

        ot_ref[u], l_ref[u] = lax.fori_loop(0, NT, pv, (zacc, zl))
        return carry

    def wait_output():
        for i in range(S // TS):
            o_copy(i).wait()

    lax.fori_loop(0, NG, functools.partial(qkv_group, True), 0)
    for c in w_copies:
        c.wait()

    def layer(n, carry):
        flag_ref[0] = 1

        def attempt(a, carry):
            @pl.when(flag_ref[0] > 0)
            def _():
                @pl.when(n + a > 0)
                def _():
                    wait_output()

                @pl.when(a == 0)
                def _():
                    ot_ref[NU - 1], l_ref[NU - 1] = lax.fori_loop(
                        0, NB // BQ, fast_block, (zacc, zl))

                @pl.when(a == 1)
                def _():
                    lax.fori_loop(0, NU, exact_unit, 0)
                    p_ref[...] = jnp.zeros(p_ref.shape, F32)

                acc = ot_ref[NU - 1]
                for m in range(NPEND):
                    v = _unpack(vt_ref[NG - 1, NT - NPEND + m, (GH - 1) * 8:GH * 8, :])
                    acc = jnp.dot(v, p_ref[m].astype(BF16),
                                  preferred_element_type=F32) + acc
                ot_ref[NU - 1] = acc
                norm_next(0, [None] * NL)
                flag_ref[0] = lax.fori_loop(
                    0, NQ, functools.partial(post_tile, n), jnp.int32(0))

            return carry

        lax.fori_loop(0, 2, attempt, 0)

        @pl.when(n == 0)
        def _():
            ln_last(NQ - 1)
            lax.fori_loop(0, NG, functools.partial(qkv_group, False), 0)

        return carry

    lax.fori_loop(0, 2, layer, 0)
    wait_output()


@jax.jit
def pallas_interleave_layers__mha_block__dense_activation_gelu__prompt_kernel(
    A_x: jax.Array,
    A_wqkv: jax.Array,
    A_wo: jax.Array,
    B_x: jax.Array,
    B_w1: jax.Array,
    B_b1: jax.Array,
    B_w2: jax.Array,
    B_b2: jax.Array,
):
    B, S, D = A_x.shape
    FF = B_w1.shape[1]
    NQ = S // TQ
    NT = S // 128
    NG = D // 128
    assert B == 1 and D == H * DH and NQ == 4 and NG == NL and TQ == 2 * TS
    hbm = pl.BlockSpec(memory_space=pl.ANY)

    out = pl.pallas_call(
        functools.partial(_kernel, S=S, D=D),
        out_shape=jax.ShapeDtypeStruct((S, D), A_x.dtype),
        in_specs=[hbm] * 7,
        out_specs=hbm,
        scratch_shapes=[
            pltpu.VMEM((S, D), BF16),
            pltpu.VMEM((NG, 2, D, 128), BF16),
            pltpu.VMEM((D, D), BF16),
            pltpu.VMEM((D, FF), BF16),
            pltpu.VMEM((FF, D), BF16),
            pltpu.VMEM((S, D), BF16),
            pltpu.VMEM((2, S, D), F32),
            pltpu.VMEM((S, D), BF16),
            pltpu.VMEM((NG, D, 128), BF16),
            pltpu.VMEM((NG, 256, D), BF16),
            pltpu.VMEM((NG, S // 2, 128), U32),
            pltpu.VMEM((NG * NQ, NL, 64, 128), U32),
            pltpu.VMEM((NG, NT, 64, 128), U32),
            pltpu.VMEM((NG, GH, NT, DH, 2, 8, 128), F32),
            pltpu.VMEM((NQ * H + 1, DH, TQ), F32),
            pltpu.VMEM((NQ * H + 1, 8, TQ), F32),
            pltpu.VMEM((TS, D), BF16),
            pltpu.VMEM((TS, D), F32),
            pltpu.VMEM((NPEND, 128, TQ), F32),
            pltpu.VMEM((NT, 128, TQ), F32),
            [pltpu.VMEM((1, NL, DH, 8, 128), F32)] * (BQ * GH),
            pltpu.VMEM((FF,), BF16),
            pltpu.VMEM((D,), BF16),
            pltpu.SMEM((1,), jnp.int32),
            pltpu.SemaphoreType.DMA((S // TS,)),
            pltpu.SemaphoreType.DMA((3 * NG,)),
            pltpu.SemaphoreType.DMA((5,)),
            pltpu.SemaphoreType.DMA((S // TS,)),
        ],
        compiler_params=pltpu.CompilerParams(vmem_limit_bytes=124 * 1024 * 1024),
    )(A_x.reshape(S, D), A_wqkv, A_wo, B_w1, B_b1, B_w2, B_b2)
    return out.reshape(B, S, D)
```

```python
import functools
import math

import jax
import jax.numpy as jnp
from jax import lax
import jax.experimental.pallas as pl
import jax.experimental.pallas.tpu as pltpu

F32 = jnp.float32
BF16 = jnp.bfloat16
U32 = jnp.uint32

H = 32
DH = 16
GH = 8
TQ = 512
TS = 256
NL = TQ // 128
BQ = 2
VR = 3
SK = 4
VLEAD = 48
QS0 = 3
NPEND = 2
KBAR_ROWS = 64
L_SAFE = 2.0 ** 64
F32_MAX = 3.0e38
EPS = 1e-5
NT_DIMS = (((1,), (1,)), ((), ()))
MXU_BLOCKS = [r for r in range(7, -1, -1) if r != VR]
NM = len(MXU_BLOCKS)


def _layernorm(x):
    m = jnp.mean(x, axis=-1, keepdims=True)
    xc = x - m
    v = jnp.mean(xc * xc, axis=-1, keepdims=True)
    return (xc * lax.rsqrt(v + EPS)).astype(BF16), v


def _gelu(x):
    c0 = math.sqrt(2.0 / math.pi)
    c1 = c0 * 0.044715
    t = jnp.tanh(x * (c0 + c1 * (x * x)))
    hx = 0.5 * x
    return hx + hx * t


def _pack(x):
    return pltpu.bitcast(x.astype(BF16), U32)


def _unpack(w):
    return pltpu.bitcast(w, BF16)


def _after(idx, y, v):
    never = lax.broadcasted_iota(jnp.int32, v.shape, 0) > (idx + v.shape[0])
    return jnp.where(never, y.reshape(v.shape), v)


def _bcast_rows(x):
    return jnp.stack([jnp.broadcast_to(x[d:d + 1], (8, 128)) for d in range(8)])


def _kernel(x_hbm, wqkv_hbm, wo_hbm, w1_hbm, b1_hbm, w2_hbm, b2_hbm, o_hbm,
            x_ref, wqv_ref, wo_ref, w1_ref, w2_ref, o_ref,
            xr_ref, xn_ref, wk_ref, wqvt_ref, k_ref, qt_ref, vt_ref, kb_ref,
            ot_ref, l_ref, ob_ref, xl_ref, p_ref, s_ref, qb_refs, b1_ref, b2_ref,
            flag_ref, sem_x, sem_g, sem_w, sem_o, *, S, D):
    NQ = S // TQ
    NU = NQ * H
    NT = S // 128
    NG = D // 128
    NB = NQ * NG
    NSUB = TQ // TS
    KV0 = NT * NM * 8
    qscale = (DH ** -0.5) * math.log2(math.e)

    def rows_of(i, sub):
        return pl.ds(pl.multiple_of(i * TQ + sub * TS, TS), TS)

    def x_copy(i):
        rows = pl.ds(pl.multiple_of(i * TS, TS), TS)
        return pltpu.make_async_copy(x_hbm.at[rows, :], x_ref.at[rows, :], sem_x.at[i])

    def o_copy(i):
        rows = pl.ds(pl.multiple_of(i * TS, TS), TS)
        return pltpu.make_async_copy(o_ref.at[rows, :], o_hbm.at[rows, :], sem_o)

    def g_copy(g, n):
        dst = wk_ref.at[g] if n == 0 else wqv_ref.at[g, n - 1]
        col = pl.multiple_of((D, 0, 2 * D)[n] + g * 128, 128)
        return pltpu.make_async_copy(
            wqkv_hbm.at[:, pl.ds(col, 128)], dst, sem_g.at[g])

    w_copies = [
        pltpu.make_async_copy(src, dst, sem_w)
        for src, dst in [(wo_hbm, wo_ref), (w1_hbm, w1_ref), (w2_hbm, w2_ref),
                         (b1_hbm, b1_ref), (b2_hbm, b2_ref)]
    ]

    def init_rows(i, carry):
        x_copy(i).wait()
        rows = pl.ds(pl.multiple_of(i * TS, TS), TS)
        x = x_ref[rows, :].astype(F32)
        xr_ref[0, rows, :] = x
        xn_ref[rows, :] = _layernorm(x)[0]
        return carry

    for i in range(S // TS):
        x_copy(i).start()
    for n in range(3):
        g_copy(0, n).start()
    xl_ref[...] = jnp.zeros(xl_ref.shape, F32)
    p_ref[...] = jnp.zeros(p_ref.shape, F32)
    lax.fori_loop(0, S // TS, init_rows, 0)
    for g in range(1, NG):
        for n in range(3):
            g_copy(g, n).start()
    for c in w_copies:
        c.start()

    def xn_blocks(blocks):
        return jnp.concatenate(
            [xn_ref[k * 128 + r * 16:k * 128 + r * 16 + 16, :] for k, r in blocks], axis=0)

    def qkv_group(first, g, carry):
        if first:
            for n in range(3):
                g_copy(g, n).wait()
            for n in range(2):
                wqvt_ref[g, n * 128:(n + 1) * 128, :] = (
                    wqv_ref[g, n].astype(F32).T.astype(BF16))
        kv = jnp.dot(xn_blocks([(k, VR) for k in range(NT)]), wk_ref[g],
                     preferred_element_type=F32)
        kbar = jnp.mean(kv[0:KBAR_ROWS], axis=0, keepdims=True)
        kv = kv - kbar
        k_ref[g, KV0:KV0 + NT * 8, :] = _pack(kv)
        kr = pltpu.bitcast(kv.astype(BF16).astype(F32), U32).reshape(NT, 16, 128)
        src = kr[:, 8:16] | lax.shift_right_logical(kr[:, 0:8], jnp.uint32(16))
        srct = src.reshape(NT * 8, 128).T
        for lane in range(128):
            row = jnp.broadcast_to(srct[lane:lane + 1], (8, NT * 8))
            col = jnp.concatenate([row] * 16, axis=0).T
            lo = pltpu.bitcast(lax.shift_left(col, jnp.uint32(16)), F32)
            hi = pltpu.bitcast(col & jnp.uint32(0xFFFF0000), F32)
            kb_ref[g, lane // DH, :, lane % DH, 0] = lo.reshape(NT, 8, 128)
            kb_ref[g, lane // DH, :, lane % DH, 1] = hi.reshape(NT, 8, 128)
        for i in range(NQ):
            xm = xn_blocks([(k, r) for k in range(i * NL, (i + 1) * NL) for r in MXU_BLOCKS])
            km = jnp.dot(xm, wk_ref[g], preferred_element_type=F32) - kbar
            k_ref[g, i * NL * NM * 8:(i + 1) * NL * NM * 8, :] = _pack(km)
        qvs = []
        for i in range(NQ):
            qvt = lax.dot_general(wqvt_ref[g], xn_ref[i * TQ:(i + 1) * TQ, :], NT_DIMS,
                                  preferred_element_type=F32)
            qvs.append(qvt)
            for a in range(NL):
                cols = slice(a * 128, (a + 1) * 128)
                qt_ref[g * NQ + i, a] = _pack(qvt[0:128, cols] * qscale)
                vt_ref[g, i * NL + a] = _pack(qvt[128:256, cols])
            if i == BQ - 1:
                rows = jnp.concatenate(
                    [_unpack(qt_ref[b, g]).astype(F32) for b in range(BQ)], axis=0)
        pace = [(i, a, r) for i in range(BQ, NQ) for a in range(NL) for r in range(32)]
        for n in range(BQ * 16):
            i, a, r = pace[(n * len(pace)) // (BQ * 16)]
            y = qvs[i][r * 8:(r + 1) * 8, a * 128:(a + 1) * 128]
            qb_refs[n // 2][0, g, (n % 2) * 8:(n % 2) * 8 + 8] = _bcast_rows(
                _after(g, y, rows[n * 8:(n + 1) * 8]))
        return carry

    def norm_cols(i, c, y=None):
        units = pl.ds(pl.multiple_of(i * H, H), H)
        cols = slice(c * 128, (c + 1) * 128)
        l = l_ref[units, :, cols]
        if y is not None:
            l = _after(i, y, l)
        ls = jnp.sum(l, axis=1, keepdims=True)
        r = pl.reciprocal(ls, approx=True)
        r = r * (2.0 - ls * r)
        r = jnp.where(jnp.maximum(ls, r) <= L_SAFE, r, jnp.nan)
        return (ot_ref[units, :, cols] * r).reshape(D, 128).T

    def norm_next(i, ys):
        for c in range(TS // 128):
            ob_ref[c * 128:(c + 1) * 128, :] = norm_cols(i, c, ys[c]).astype(BF16)

    def ln_last(i, y=None):
        x = xl_ref[...]
        if y is not None:
            x = jnp.concatenate([_after(i, y, x[:, 0:128]), x[:, 128:]], axis=1)
        xn_ref[rows_of(i, NSUB - 1), :] = _layernorm(x)[0]

    def post_tile(n, i, bad):
        b1 = b1_ref[...].astype(F32)
        b2 = b2_ref[...].astype(F32)

        def col(y, c):
            return y[:, c * 128:(c + 1) * 128]

        x1 = []
        for sub in range(NSUB):
            if sub == 0:
                o = ob_ref[...]
            else:
                o = jnp.concatenate(
                    [norm_cols(i, TS // 128 + c, col(x1[0], c)) for c in range(TS // 128)],
                    axis=0).astype(BF16)
            x1.append(jnp.dot(o, wo_ref[...], preferred_element_type=F32)
                      + xr_ref[n, rows_of(i, sub), :])
        hh = []
        for sub in range(NSUB):
            xn, var = _layernorm(x1[sub])
            bad = jnp.maximum(bad, jnp.max(jnp.where(var <= F32_MAX, 0, 1)))
            h = jnp.dot(xn, w1_ref[...], preferred_element_type=F32) + b1
            hh.append(_gelu(h).astype(BF16))
        x2 = [jnp.dot(hh[sub], w2_ref[...], preferred_element_type=F32) + (x1[sub] + b2)
              for sub in range(NSUB)]
        ln_last(jnp.maximum(i - 1, 0), col(x2[0], 0))
        norm_next(jnp.minimum(i + 1, NQ - 1), [col(x2[0], 1), col(x2[0], 2)])
        for sub in range(NSUB):
            o_ref[rows_of(i, sub), :] = x2[sub].astype(o_ref.dtype)
            o_copy(i * NSUB + sub).start()
            xr_ref[1 - n, rows_of(i, sub), :] = x2[sub]
            if sub < NSUB - 1:
                xn_ref[rows_of(i, sub), :] = _layernorm(x2[sub])[0]
            else:
                xl_ref[...] = x2[sub]
        return bad

    zacc = jnp.zeros((DH, TQ), F32)
    zl = jnp.zeros((8, TQ), F32)

    def tile_rows(blocks):
        return jnp.concatenate([blocks[r] for r in range(8)], axis=0)

    def rowsum(p):
        return jnp.sum(p.reshape(p.shape[0] // 8, 8, TQ), axis=0)

    bounds = [0] + [NM * k - SK for k in range(1, NT + 1)] + [NM * NT]
    period = 16 * (NM + 1)
    vat = 7 - VR

    def fast_block(tb, carry):
        acc, lprev = carry
        t = tb * BQ
        g = lax.shift_right_logical(t, 2)
        i = t & (NQ - 1)
        tn = jnp.minimum(t + BQ, NB - BQ)
        tp = jnp.maximum(t - 1, 0)
        gprev = lax.shift_right_logical(tp, 2)
        slot_prev = jnp.where(t == 0, NU, (tp & (NQ - 1)) * H + gprev * GH + (GH - 1))

        queue = [(-1, NT - NPEND + n, p_ref[n]) for n in range(NPEND)]
        lsum = {-1: lprev}
        done = []
        clock = 0
        uniq = 0

        def result_at(when):
            cand = [e for e in done if e[0] <= when]
            if not cand:
                return None
            return cand[-1][1][cand[-1][2]:cand[-1][2] + 8, 0:128]

        def add_l(u, p):
            lsum[u] = p if lsum[u] is None else lsum[u] + p

        def make_qb(u, part, y):
            lt, half = divmod(part, 2)
            j = u % GH
            src = _unpack(qt_ref[tn + u // GH, lt, 8 * j:8 * j + 8, :]).astype(F32)
            qb_refs[u][0, lt, half * 8:half * 8 + 8] = _bcast_rows(
                _after(t, y, src[half * 8:half * 8 + 8]))

        for u in range(BQ * GH):
            hb, j = divmod(u, GH)
            parts = [jnp.zeros((16 * j, TQ), BF16)] if j > 0 else []
            parts.append(_unpack(jnp.concatenate(
                [qt_ref[t + hb, a, 8 * j:8 * j + 8, :] for a in range(NL)], axis=1)))
            if j < GH - 1:
                parts.append(jnp.zeros((16 * (GH - 1 - j), TQ), BF16))
            qm = jnp.concatenate(parts, axis=0)
            lsum[u] = None
            blocks = {}
            for si in range(NT + 1):
                lo, hi = bounds[si], bounds[si + 1]
                s = jnp.dot(_unpack(k_ref[g, lo * 8:hi * 8, :]), qm,
                            preferred_element_type=F32)
                e = jnp.exp2(s)
                for n in range(lo, hi):
                    k, pos = divmod(n, NM)
                    if pos == vat:
                        cols = []
                        for lt in range(NL):
                            uniq += 1
                            tq = jnp.minimum(t, 1000 + uniq)
                            qb = qb_refs[u][tq - t, lt]
                            y = result_at(clock - VLEAD - ((NL - 1 - lt) * period) // NL)
                            if y is not None:
                                qb = jnp.concatenate(
                                    [_after(t, y, qb[0])[None], qb[1:]], axis=0)
                            kb = kb_ref[lax.shift_right_logical(tq, 2), j, k]
                            cols.append(jnp.sum(kb * qb[:, None], axis=0))
                        ev = jnp.exp2(jnp.concatenate(cols, axis=2))
                        add_l(u, ev[0] + ev[1])
                        blocks[VR] = ev.reshape(16, TQ)
                    row = (n - lo) * 16
                    done.append((clock, s, row))
                    done.append((clock + 8, s, row + 8))
                    clock += 16
                    blocks[MXU_BLOCKS[pos]] = e[row:row + 16]
                    add_l(u, e[row:row + 8] + e[row + 8:row + 16])
                    if pos == NM - 1:
                        queue.append((u, k, tile_rows(blocks)))
                        blocks = {}
                done = done[-48:]
                if u > 0 and QS0 <= si < QS0 + 2 * NL:
                    make_qb(u - 1, si - QS0, result_at(clock))
                if si < NT:
                    ua, k, p = queue.pop(0)
                    ga, ja = (gprev, GH - 1) if ua < 0 else (g, ua % GH)
                    v = _unpack(vt_ref[ga, k, ja * 8:(ja + 1) * 8, :])
                    pv = jnp.dot(v, p.astype(BF16), preferred_element_type=F32)
                    acc = pv if acc is None else pv + acc
                    done.append((clock, acc, 0))
                    done.append((clock + 8, acc, 8))
                    clock += 16
                    if k == NT - 1:
                        slot = slot_prev if ua < 0 else (i + ua // GH) * H + g * GH + ja
                        ot_ref[slot] = acc
                        l_ref[slot] = lsum[ua]
                        acc = None
        assert [e[:2] for e in queue] == [
            (BQ * GH - 1, NT - NPEND + n) for n in range(NPEND)]
        for n in range(NPEND):
            p_ref[n] = queue[n][2]
        for part in range(2 * NL):
            make_qb(BQ * GH - 1, part, result_at(clock - 128 + 8 * part))
        return acc, lsum[BQ * GH - 1]

    def exact_unit(u, carry):
        i = lax.shift_right_logical(u, 5)
        h = u & (H - 1)
        g = lax.shift_right_logical(h, 3)
        j = h & (GH - 1)
        w = jnp.concatenate([qt_ref[g * NQ + i, a] for a in range(NL)], axis=1)
        row = lax.broadcasted_iota(jnp.int32, w.shape, 0)
        qm = _unpack(jnp.where(lax.shift_right_logical(row, 3) == j, w, jnp.uint32(0)))

        def score(k, mx):
            kk = jnp.concatenate(
                [k_ref[g, pl.ds(pl.multiple_of(k * (NM * 8), 8), NM * 8), :],
                 k_ref[g, pl.ds(pl.multiple_of(KV0 + k * 8, 8), 8), :]], axis=0)
            sc = jnp.dot(_unpack(kk), qm, preferred_element_type=F32)
            s_ref[k] = tile_rows({r: sc[n * 16:(n + 1) * 16]
                                  for n, r in enumerate(MXU_BLOCKS + [VR])})
            return jnp.maximum(mx, jnp.max(sc.reshape(16, 8, TQ), axis=0))

        mx = lax.fori_loop(0, NT, score, jnp.full((8, TQ), -jnp.inf, F32))
        m = jnp.max(mx, axis=0, keepdims=True)

        def pv(k, st):
            p = jnp.exp2(s_ref[k] - m)
            v = _unpack(vt_ref[g, k, pl.ds(pl.multiple_of(j * 8, 8), 8), :])
            return (jnp.dot(v, p.astype(BF16), preferred_element_type=F32) + st[0],
                    st[1] + rowsum(p))

        ot_ref[u], l_ref[u] = lax.fori_loop(0, NT, pv, (zacc, zl))
        return carry

    def wait_output():
        for i in range(S // TS):
            o_copy(i).wait()

    lax.fori_loop(0, NG, functools.partial(qkv_group, True), 0)
    for c in w_copies:
        c.wait()

    def layer(n, carry):
        flag_ref[0] = 1

        def attempt(a, carry):
            @pl.when(flag_ref[0] > 0)
            def _():
                @pl.when(n + a > 0)
                def _():
                    wait_output()

                @pl.when(a == 0)
                def _():
                    ot_ref[NU - 1], l_ref[NU - 1] = lax.fori_loop(
                        0, NB // BQ, fast_block, (zacc, zl))

                @pl.when(a == 1)
                def _():
                    lax.fori_loop(0, NU, exact_unit, 0)
                    p_ref[...] = jnp.zeros(p_ref.shape, F32)

                acc = ot_ref[NU - 1]
                for m in range(NPEND):
                    v = _unpack(vt_ref[NG - 1, NT - NPEND + m, (GH - 1) * 8:GH * 8, :])
                    acc = jnp.dot(v, p_ref[m].astype(BF16),
                                  preferred_element_type=F32) + acc
                ot_ref[NU - 1] = acc
                norm_next(0, [None] * NL)
                flag_ref[0] = lax.fori_loop(
                    0, NQ, functools.partial(post_tile, n), jnp.int32(0))

            return carry

        lax.fori_loop(0, 2, attempt, 0)

        @pl.when(n == 0)
        def _():
            ln_last(NQ - 1)
            lax.fori_loop(0, NG, functools.partial(qkv_group, False), 0)

        return carry

    lax.fori_loop(0, 2, layer, 0)
    wait_output()


@jax.jit
def pallas_interleave_layers__mha_block__dense_activation_gelu__prompt_kernel(
    A_x: jax.Array,
    A_wqkv: jax.Array,
    A_wo: jax.Array,
    B_x: jax.Array,
    B_w1: jax.Array,
    B_b1: jax.Array,
    B_w2: jax.Array,
    B_b2: jax.Array,
):
    B, S, D = A_x.shape
    FF = B_w1.shape[1]
    NQ = S // TQ
    NT = S // 128
    NG = D // 128
    assert B == 1 and D == H * DH and NQ == 4 and NG == NL and TQ == 2 * TS
    hbm = pl.BlockSpec(memory_space=pl.ANY)

    out = pl.pallas_call(
        functools.partial(_kernel, S=S, D=D),
        out_shape=jax.ShapeDtypeStruct((S, D), A_x.dtype),
        in_specs=[hbm] * 7,
        out_specs=hbm,
        scratch_shapes=[
            pltpu.VMEM((S, D), BF16),
            pltpu.VMEM((NG, 2, D, 128), BF16),
            pltpu.VMEM((D, D), BF16),
            pltpu.VMEM((D, FF), BF16),
            pltpu.VMEM((FF, D), BF16),
            pltpu.VMEM((S, D), BF16),
            pltpu.VMEM((2, S, D), F32),
            pltpu.VMEM((S, D), BF16),
            pltpu.VMEM((NG, D, 128), BF16),
            pltpu.VMEM((NG, 256, D), BF16),
            pltpu.VMEM((NG, S // 2, 128), U32),
            pltpu.VMEM((NG * NQ, NL, 64, 128), U32),
            pltpu.VMEM((NG, NT, 64, 128), U32),
            pltpu.VMEM((NG, GH, NT, DH, 2, 8, 128), F32),
            pltpu.VMEM((NQ * H + 1, DH, TQ), F32),
            pltpu.VMEM((NQ * H + 1, 8, TQ), F32),
            pltpu.VMEM((TS, D), BF16),
            pltpu.VMEM((TS, D), F32),
            pltpu.VMEM((NPEND, 128, TQ), F32),
            pltpu.VMEM((NT, 128, TQ), F32),
            [pltpu.VMEM((1, NL, DH, 8, 128), F32)] * (BQ * GH),
            pltpu.VMEM((FF,), BF16),
            pltpu.VMEM((D,), BF16),
            pltpu.SMEM((1,), jnp.int32),
            pltpu.SemaphoreType.DMA((S // TS,)),
            pltpu.SemaphoreType.DMA((NG,)),
            pltpu.SemaphoreType.DMA(()),
            pltpu.SemaphoreType.DMA(()),
        ],
        compiler_params=pltpu.CompilerParams(vmem_limit_bytes=124 * 1024 * 1024),
    )(A_x.reshape(S, D), A_wqkv, A_wo, B_w1, B_b1, B_w2, B_b2)
    return out.reshape(B, S, D)
```
